```python
import os as _os
_os.environ.setdefault('JAX_PLATFORMS', 'cpu')
import jax
import jax.numpy as jnp

def _softmax(x, axis=-1):
    return jax.nn.softmax(x, axis=axis)

def _gelu(x):
    return jax.nn.gelu(x, approximate=True)

def _silu(x):
    return jax.nn.silu(x)

def _sigmoid(x):
    return jax.nn.sigmoid(x)

def _layernorm(x, axis=-1, eps=1e-05):
    m = jnp.mean(x, axis=axis, keepdims=True)
    v = jnp.var(x, axis=axis, keepdims=True)
    return (x - m) / jnp.sqrt(v + eps)

def _scatter_add(tgt, idx, src, axis=0):
    return tgt.at[idx].add(src)

def _segment_sum(src, seg, n):
    return jax.ops.segment_sum(src, seg, n)

class _Rng:

    def __init__(self, key):
        self._k = key

    def _next(self):
        self._k, sub = jax.random.split(self._k)
        return sub

    def normal(self, shape):
        return jax.random.normal(self._next(), shape, dtype=jnp.bfloat16)

    def randint(self, lo, hi, shape):
        return jax.random.randint(self._next(), shape, lo, hi, dtype=jnp.int32)

    def uniform(self, shape, lo=0.0, hi=1.0):
        return jax.random.uniform(self._next(), shape, jnp.bfloat16, lo, hi)

    def permutation(self, n):
        return jax.random.permutation(self._next(), n)
kernel_name = 'standalone__conformer_conv_module__speech'

def setup_inputs():
    _rng = _Rng(jax.random.key(int.from_bytes(__import__("os").urandom(4), "little")))
    _w = lambda a: (lambda t: t.astype(jnp.bfloat16) if jnp.issubdtype(t.dtype, jnp.floating) else t)(jnp.asarray(a))
    B, T, D, K = (2, 16000, 256, 5)
    return {'x': _w((lambda *s: _rng.normal(s) * 0.2)(B, T, D)), 'w_pw1': _w((lambda *s: _rng.normal(s) * 0.2)(D, 2 * D)), 'dw': _w((lambda *s: _rng.normal(s) * 0.05)(K, D)), 'w_pw2': _w((lambda *s: _rng.normal(s) * 0.05)(D, D))}

def reference(x, w_pw1, dw, w_pw2):
    B, T, D = x.shape
    K = dw.shape[0]
    h = x @ w_pw1
    a, b = (h[..., :D].copy(), h[..., D:].copy())
    h = a * _sigmoid(b)
    pad = K // 2
    hp = jnp.pad(h, ((0, 0), (pad, pad), (0, 0)))
    out = jnp.zeros_like(h)
    for i in range(K):
        out = out + hp[:, i:i + T, :] * dw[i][None, None, :]
    return _silu(out) @ w_pw2
```

```python
import jax
import jax.numpy as jnp
import jax.experimental.pallas as pl
import jax.experimental.pallas.tpu as pltpu

TB = 2000
HB = 16


@jax.jit
def pallas_standalone__conformer_conv_module__speech_kernel(
    x: jax.Array,
    w_pw1: jax.Array,
    dw: jax.Array,
    w_pw2: jax.Array,
):
    B, T, D = x.shape
    K = dw.shape[0]
    pad = K // 2
    nT = T // TB
    nH = T // HB
    r = TB // HB

    def kernel_function(xp_ref, x_ref, xn_ref, w1_ref, dw_ref, w2_ref, o_ref, h_ref):
        j = pl.program_id(1)
        w1 = w1_ref[...]

        def glu(xv):
            hh = jnp.dot(xv, w1, preferred_element_type=jnp.float32)
            a = hh[:, :D]
            b = hh[:, D:]
            return a * jax.nn.sigmoid(b)

        hp = glu(xp_ref[0])
        hn = glu(xn_ref[0])
        hp = jnp.where(j > 0, hp, 0.0)
        hn = jnp.where(j < nT - 1, hn, 0.0)
        h_ref[0:HB, :] = hp
        h_ref[HB + TB:, :] = hn
        h_ref[HB:HB + TB, :] = glu(x_ref[0])
        dwf = dw_ref[...].astype(jnp.float32)
        acc = None
        for i in range(K):
            t = h_ref[HB - pad + i:HB - pad + i + TB, :] * dwf[i:i + 1, :]
            acc = t if acc is None else acc + t
        s = acc * jax.nn.sigmoid(acc)
        o = jnp.dot(s.astype(jnp.bfloat16), w2_ref[...], preferred_element_type=jnp.float32)
        o_ref[0] = o.astype(o_ref.dtype)

    return pl.pallas_call(
        kernel_function,
        grid=(B, nT),
        in_specs=[
            pl.BlockSpec((1, HB, D), lambda b, j: (b, jnp.maximum(j * r - 1, 0), 0)),
            pl.BlockSpec((1, TB, D), lambda b, j: (b, j, 0)),
            pl.BlockSpec((1, HB, D), lambda b, j: (b, jnp.minimum((j + 1) * r, nH - 1), 0)),
            pl.BlockSpec((D, 2 * D), lambda b, j: (0, 0)),
            pl.BlockSpec((K, D), lambda b, j: (0, 0)),
            pl.BlockSpec((D, D), lambda b, j: (0, 0)),
        ],
        out_specs=pl.BlockSpec((1, TB, D), lambda b, j: (b, j, 0)),
        out_shape=jax.ShapeDtypeStruct((B, T, D), x.dtype),
        scratch_shapes=[pltpu.VMEM((TB + 2 * HB, D), jnp.float32)],
        compiler_params=pltpu.CompilerParams(
            dimension_semantics=("arbitrary", "arbitrary"),
            vmem_limit_bytes=100 * 1024 * 1024,
        ),
    )(x, x, x, w_pw1, dw, w_pw2)
```

```python
import contextlib
import jax
import jax.numpy as jnp
from jax import lax
import jax.experimental.pallas as pl
import jax.experimental.pallas.tpu as pltpu

MS = 400
UN = 22
PRO = (1, 1, 3, 8)
EPI = (2,)
TAILSPLIT = 25
TAILN = 2
ODEFER = 12
RAW0 = True
SCOPES = False


def scope(nm):
    return jax.named_scope(nm) if SCOPES else contextlib.nullcontext()


@jax.jit
def pallas_standalone__conformer_conv_module__speech_kernel(x, w_pw1, dw, w_pw2):
    B, T, D = x.shape
    K = dw.shape[0]
    pad = K // 2
    L = 128
    NC = D // L
    m = MS
    U = UN
    n = T // m
    S = B * n
    NT = S + 1
    P = sum(PRO)
    E = sum(EPI)
    NI = (NT - P - E) // U
    assert T % m == 0 and P + E + NI * U == NT and U % 2 == 0 and m % 16 == 0, (NT, P, E, NI)
    assert ODEFER <= P - 1 and EPI[-1] >= 1
    starts = []
    t = 0
    for c in PRO:
        starts.append((t, c)); t += c
    loop0 = t
    t += NI * U
    epi = []
    for c in EPI:
        epi.append((t, c)); t += c
    R = B * T
    f32 = jnp.float32
    bf16 = jnp.bfloat16
    NP = len(starts)

    def kernel(x_hbm, w1_hbm, dw_hbm, w2_hbm, o_hbm, xb, ob, hb, w1b, w1s, w2b, dwb, xsem, osem, bsem):
        def mult(v, k):
            return v if isinstance(v, int) else pl.multiple_of(v, k)

        def x_copy(s, cnt, sem):
            rows = pl.ds(mult(s * m, m), cnt * m)
            return pltpu.make_async_copy(x_hbm.at[rows], xb.at[rows], sem)

        def x_load(s):
            return xb[pl.ds(mult(s * m, m), m), :]

        w1_cp = pltpu.make_async_copy(w1_hbm, w1b, xsem.at[0])
        w2_cp = pltpu.make_async_copy(w2_hbm, w2b, xsem.at[1])
        dw_cp = pltpu.make_async_copy(dw_hbm, dwb, xsem.at[1])

        def w1_load(ref, c):
            return jnp.concatenate([ref[:, c * L:(c + 1) * L], ref[:, D + c * L:D + (c + 1) * L]], axis=1)

        def o_copy(r0, nr):
            rows = pl.ds(r0, nr)
            return pltpu.make_async_copy(ob.at[rows], o_hbm.at[rows], osem)

        def xrange_of(t0, cnt):
            return (t0, min(t0 + cnt, S) - t0)

        def order():
            pl.semaphore_signal(bsem, 1)
            pl.semaphore_wait(bsem, 1)

        for ri, (t0, cnt) in enumerate(starts):
            if ri == 0:
                w1_cp.start()
            x_copy(*xrange_of(t0, cnt), xsem.at[ri]).start()
            if ri == 1:
                dw_cp.start()
                w2_cp.start()
            order()
        for i in range(NI):
            x_copy(loop0 + i * U, U, xsem.at[NP + i]).start()
            order()
        ne = 0
        for ri, (t0, cnt) in enumerate(epi):
            lo, c = xrange_of(t0, cnt)
            if c > 0:
                x_copy(lo, c, xsem.at[NP + NI + ri]).start()

        zero = jnp.zeros((8, L), f32)

        def stage1(s, cur, first):
            prev = 1 - cur
            boundary = (s % n) == 0

            def keep(v):
                if isinstance(boundary, bool):
                    return zero if boundary else v
                return jnp.where(boundary, zero, v)
            for c in range(NC):
                if isinstance(boundary, bool) and boundary:
                    hb[cur, c, 0:8, :] = zero
                else:
                    hb[cur, c, 0:8, :] = keep(hb[prev, c, m:m + 8, :])
            xv = x_load(s)
            for c in range(NC):
                if first and RAW0:
                    hh = jnp.dot(xv, w1_load(w1b, c), preferred_element_type=f32) * 0.5
                else:
                    hh = jnp.dot(xv, w1_load(w1s, c), preferred_element_type=f32)
                a = hh[:, :L]
                b = hh[:, L:]
                h = a + a * jnp.tanh(b)
                hb[cur, c, 8:8 + m, :] = h
                if not first:
                    hb[prev, c, 8 + m:16 + m, :] = keep(h[0:8])

        def stage2(s, slot, nsplit=1):
            dwf = dwb[...].astype(f32) * 0.5
            ss = []
            for c in range(NC):
                acc = None
                for i in range(K):
                    tt = hb[slot, c, 8 - pad + i:8 - pad + i + m, :] * dwf[i:i + 1, c * L:(c + 1) * L]
                    acc = tt if acc is None else acc + tt
                ss.append(acc + acc * jnp.tanh(acc))
            sv = jnp.concatenate(ss, axis=1).astype(bf16)
            o = jnp.dot(sv, w2b[...], preferred_element_type=f32).astype(bf16)
            base = mult(s * m, m)
            mm = m // nsplit
            for q in range(nsplit):
                r0 = base + q * mm
                ob[pl.ds(r0, mm), :] = o[q * mm:(q + 1) * mm]
                if isinstance(s, int) and s < ODEFER:
                    if s == ODEFER - 1 and q == nsplit - 1:
                        o_copy(0, ODEFER * m).start()
                else:
                    o_copy(r0, mm).start()

        def time_step(t, par, static_t=None):
            if static_t is not None and static_t == S:
                for c in range(NC):
                    hb[1 - par, c, 8 + m:16 + m, :] = zero
                stage2(t - 1, 1 - par, TAILSPLIT)
                return
            stage1(t, par, static_t == 0)
            if static_t is None:
                stage2(t - 1, 1 - par)
            elif static_t >= 1:
                stage2(t - 1, 1 - par, TAILSPLIT if static_t - 1 >= S - TAILN else 1)

        def run_static(regions, off):
            for ri, (t0, cnt) in enumerate(regions):
                lo, c = xrange_of(t0, cnt)
                with scope(f'wait{t0}'):
                    if c > 0:
                        x_copy(lo, c, xsem.at[off + ri]).wait()
                    if off + ri == 0:
                        w1_cp.wait()
                    if off + ri == 1:
                        dw_cp.wait()
                        w2_cp.wait()
                with scope(f'comp{t0}'):
                    if off + ri == 0 and not RAW0:
                        w1s[...] = (w1b[...].astype(f32) * 0.5).astype(bf16)
                    for tt in range(t0, t0 + cnt):
                        time_step(tt, tt % 2, tt)
                    if off + ri == 0 and RAW0:
                        w1s[...] = (w1b[...].astype(f32) * 0.5).astype(bf16)

        run_static(starts, 0)

        def body(i, carry):
            t0 = loop0 + i * U
            with scope('lwait'):
                x_copy(t0, U, xsem.at[NP + i]).wait()
            with scope('lcomp'):
                for u in range(U):
                    time_step(t0 + u, (loop0 + u) % 2)
            return carry

        if NI > 0:
            lax.fori_loop(0, NI, body, 0)
        run_static(epi, NP + NI)
        with scope('final'):
            pltpu.make_async_copy(ob, o_hbm, osem).wait()

    xf = x.reshape(R, D)
    nsem = NP + NI + sum(1 for (t0, cnt) in epi if min(t0 + cnt, S) - t0 > 0)
    out = pl.pallas_call(
        kernel,
        grid=(),
        in_specs=[pl.BlockSpec(memory_space=pl.ANY)] * 4,
        out_specs=pl.BlockSpec(memory_space=pl.ANY),
        out_shape=jax.ShapeDtypeStruct((R, D), x.dtype),
        scratch_shapes=[
            pltpu.VMEM((R, D), bf16),
            pltpu.VMEM((R, D), bf16),
            pltpu.VMEM((2, NC, m + 16, L), f32),
            pltpu.VMEM((D, 2 * D), bf16),
            pltpu.VMEM((D, 2 * D), bf16),
            pltpu.VMEM((D, D), bf16),
            pltpu.VMEM((K, D), dw.dtype),
            pltpu.SemaphoreType.DMA((nsem,)),
            pltpu.SemaphoreType.DMA(()),
            pltpu.SemaphoreType.REGULAR,
        ],
        compiler_params=pltpu.CompilerParams(vmem_limit_bytes=100 * 1024 * 1024),
    )(xf, w_pw1, dw, w_pw2)
    return out.reshape(B, T, D)
```

```python
import jax
import jax.numpy as jnp
from jax import lax
import jax.experimental.pallas as pl
import jax.experimental.pallas.tpu as pltpu

MS = 400
UN = 38
EPI = 2
RD = 4
TAILN = 2
TAILSPLIT = 25
X0A = 192
NPRO = 3
PINW = 16


@jax.jit
def pallas_standalone__conformer_conv_module__speech_kernel(
    x: jax.Array,
    w_pw1: jax.Array,
    dw: jax.Array,
    w_pw2: jax.Array,
):
    B, T, D = x.shape
    K = dw.shape[0]
    pad = K // 2
    L = 128
    NC = D // L
    m = MS
    U = UN
    n = T // m
    S = B * n
    NT = S + 1
    P = NPRO
    NI = (NT - P - EPI) // U
    assert T % m == 0 and m % 16 == 0 and D % L == 0 and pad <= 8
    assert P + NI * U + EPI == NT and U % 2 == 0 and EPI >= TAILN and S > RD + 1
    assert P >= 2 and RD == 4 and 0 < X0A < m
    R = B * T
    f32 = jnp.float32
    bf16 = jnp.bfloat16

    loop0 = P
    epi0 = loop0 + NI * U

    def kernel_function(x_hbm, w1_hbm, dw_hbm, w2_hbm, o_hbm,
                        xb, ob, hb, w1b, w1s, w2b, dwb, xsem, osem, bsem):
        def mult(v, k):
            return v if isinstance(v, int) else pl.multiple_of(v, k)

        def x_rows(r0, nr, sem):
            rows = pl.ds(r0, nr)
            return pltpu.make_async_copy(x_hbm.at[rows], xb.at[rows], sem)

        def x_copy(s, cnt, sem):
            return x_rows(mult(s * m, m), cnt * m, sem)

        def o_copy(r0, nr):
            rows = pl.ds(r0, nr)
            return pltpu.make_async_copy(ob.at[rows], o_hbm.at[rows], osem)

        def order():
            pl.semaphore_signal(bsem, 1)
            pl.semaphore_wait(bsem, 1)

        w1_cp = pltpu.make_async_copy(w1_hbm, w1b, xsem.at[2])
        x0a_cp = x_rows(0, X0A, xsem.at[2])
        x0b_cp = x_rows(X0A, m - X0A, xsem.at[3])
        w2_cp = pltpu.make_async_copy(w2_hbm, w2b.at[0:D], xsem.at[0])
        dw_cp = pltpu.make_async_copy(dw_hbm, dwb, xsem.at[0])

        def ring(s):
            return x_copy(s, 1, xsem.at[s % RD])

        def ring_wait(s):
            ring(s).wait()
            if isinstance(s, int):
                if s + RD < S:
                    ring(s + RD).start()
            else:
                @pl.when(s + RD < S)
                def _():
                    ring(s + RD).start()

        def anchor(ref, r0, v):
            ref[r0:r0 + 16, :] = v

        def w1_cols(ref, c):
            return jnp.concatenate(
                [ref[:, c * L:(c + 1) * L], ref[:, D + c * L:D + (c + 1) * L]], axis=1)

        def glu(hh):
            a = hh[:, :L]
            return a + a * jnp.tanh(hh[:, L:])

        zero = jnp.zeros((8, L), f32)

        def stage1_first():
            for c in range(NC):
                hb[0, c, 0:8, :] = zero
            w0 = w1_cols(w1b, 0)
            h = glu(jnp.dot(xb[0:X0A, :], w0, preferred_element_type=f32) * 0.5)
            hb[0, 0, 8:8 + X0A, :] = h
            v = h[0:16].astype(bf16)
            anchor(xb, R, jnp.concatenate([v, v], axis=1))
            x0b_cp.wait()
            ring(3).start()
            hb[0, 0, 8 + X0A:8 + m, :] = glu(
                jnp.dot(xb[X0A:m, :], w0, preferred_element_type=f32) * 0.5)
            for c in range(1, NC):
                h = glu(jnp.dot(xb[0:m, :], w1_cols(w1b, c), preferred_element_type=f32) * 0.5)
                hb[0, c, 8:8 + m, :] = h

        def stage1(s, cur, after=None):
            prev = 1 - cur
            boundary = (s % n) == 0

            def keep(v):
                if isinstance(boundary, bool):
                    return zero if boundary else v
                return jnp.where(boundary, zero, v)

            for c in range(NC):
                hb[cur, c, 0:8, :] = keep(hb[prev, c, m:m + 8, :])
            xv = xb[pl.ds(mult(s * m, m), m), :]
            for c in range(NC):
                h = glu(jnp.dot(xv, w1_cols(w1s, c), preferred_element_type=f32))
                hb[cur, c, 8:8 + m, :] = h
                hb[prev, c, 8 + m:16 + m, :] = keep(h[0:8])
            if after is not None:
                v = h[PINW:PINW + 16].astype(bf16)
                after(jnp.concatenate([v, v], axis=1))

        def stage2(s, slot, nsplit):
            dwf = dwb[...].astype(f32) * 0.5
            ss = []
            for c in range(NC):
                acc = None
                for i in range(K):
                    tap = hb[slot, c, 8 - pad + i:8 - pad + i + m, :] * dwf[i:i + 1, c * L:(c + 1) * L]
                    acc = tap if acc is None else acc + tap
                ss.append(acc + acc * jnp.tanh(acc))
            sv = jnp.concatenate(ss, axis=1).astype(bf16)
            o = jnp.dot(sv, w2b[0:D], preferred_element_type=f32).astype(bf16)
            base = mult(s * m, m)
            mm = m // nsplit
            for q in range(nsplit):
                r0 = base + q * mm
                ob[pl.ds(r0, mm), :] = o[q * mm:(q + 1) * mm]
                o_copy(r0, mm).start()

        w1_cp.start()
        x0a_cp.start()
        order()
        x0b_cp.start()
        order()
        ring(1).start()
        order()
        dw_cp.start()
        w2_cp.start()

        w1_cp.wait()
        x0a_cp.wait()
        ring(2).start()

        def after0(v):
            anchor(w2b, D, v)
            dw_cp.wait()
            w2_cp.wait()
            ring(4).start()

        stage1_first()
        w1s[...] = (w1b[...].astype(f32) * 0.5).astype(bf16)
        for tt in range(1, P):
            ring_wait(tt)
            stage1(tt, tt % 2, after0 if tt == 1 else None)
            stage2(tt - 1, 1 - tt % 2, 1)

        def body(i, carry):
            t0 = loop0 + i * U
            for u in range(U):
                par = (loop0 + u) % 2
                ring_wait(t0 + u)
                stage1(t0 + u, par)
                stage2(t0 + u - 1, 1 - par, 1)
            return carry

        lax.fori_loop(0, NI, body, 0)

        for tt in range(epi0, NT):
            par = tt % 2
            if tt < S:
                ring_wait(tt)
                stage1(tt, par)
            else:
                for c in range(NC):
                    hb[1 - par, c, 8 + m:16 + m, :] = zero
            stage2(tt - 1, 1 - par, TAILSPLIT if tt - 1 >= S - TAILN else 1)
        pltpu.make_async_copy(ob, o_hbm, osem).wait()

    out = pl.pallas_call(
        kernel_function,
        grid=(),
        in_specs=[pl.BlockSpec(memory_space=pl.ANY)] * 4,
        out_specs=pl.BlockSpec(memory_space=pl.ANY),
        out_shape=jax.ShapeDtypeStruct((R, D), x.dtype),
        scratch_shapes=[
            pltpu.VMEM((R + 16, D), x.dtype),
            pltpu.VMEM((R, D), x.dtype),
            pltpu.VMEM((2, NC, m + 16, L), f32),
            pltpu.VMEM((D, 2 * D), w_pw1.dtype),
            pltpu.VMEM((D, 2 * D), w_pw1.dtype),
            pltpu.VMEM((D + 16, D), w_pw2.dtype),
            pltpu.VMEM((K, D), dw.dtype),
            pltpu.SemaphoreType.DMA((RD,)),
            pltpu.SemaphoreType.DMA(()),
            pltpu.SemaphoreType.REGULAR,
        ],
        compiler_params=pltpu.CompilerParams(
            vmem_limit_bytes=64 * 1024 * 1024,
            flags={"XLA_TPU_RESCHEDULE_DMA_DONES": True},
        ),
    )(x.reshape(R, D), w_pw1, dw, w_pw2)
    return out.reshape(B, T, D)
```
